```python
import jax
import jax.numpy as jnp

def _softmax(x, axis=-1):
    return jax.nn.softmax(x, axis=axis)
def _gelu(x):
    return jax.nn.gelu(x, approximate=True)
def _silu(x):
    return jax.nn.silu(x)
def _sigmoid(x):
    return jax.nn.sigmoid(x)
def _layernorm(x, axis=-1, eps=1e-5):
    m = jnp.mean(x, axis=axis, keepdims=True)
    v = jnp.var(x, axis=axis, keepdims=True)
    return (x - m) / jnp.sqrt(v + eps)
def _scatter_add(tgt, idx, src, axis=0):
    return tgt.at[idx].add(src)
def _segment_sum(src, seg, n):
    return jax.ops.segment_sum(src, seg, n)
class _Rng:
    def __init__(self, key):
        self._k = key
    def _next(self):
        self._k, sub = jax.random.split(self._k)
        return sub
    def normal(self, shape):
        return jax.random.normal(self._next(), shape, dtype=jnp.bfloat16)
    def randint(self, lo, hi, shape):
        return jax.random.randint(self._next(), shape, lo, hi, dtype=jnp.int32)
    def uniform(self, shape, lo=0.0, hi=1.0):
        return jax.random.uniform(self._next(), shape, jnp.bfloat16, lo, hi)
    def permutation(self, n):
        return jax.random.permutation(self._next(), n)


kernel_name = 'sequential_preLN__compressed_kv_cla__moe_arch_mod__prompt'

def setup_inputs():
    _rng = _Rng(jax.random.key(int.from_bytes(__import__("os").urandom(4), "little")))
    _w = (lambda a: (lambda t: t.astype(jnp.bfloat16) if jnp.issubdtype(t.dtype, jnp.floating) else t)(jnp.asarray(a)))
    def _A_setup():
        B, H, Sq, Sk, D, M = 1, 32, 2048, 2048, 128, 1024
        Dc = 4 * D
        return {
            "x": _w((lambda *s: _rng.normal(s) * 0.05)(B, Sq, M)),
            "c_kv": _w((lambda *s: _rng.normal(s) * 0.05)(B, Sk, Dc)),
            "w_q": _w((lambda *s: _rng.normal(s) * 0.05)(M, H, D) * (M ** -0.5)),
            "w_uk": _w((lambda *s: _rng.normal(s) * 0.05)(Dc, H, D) * (Dc ** -0.5)),
            "w_uv": _w((lambda *s: _rng.normal(s) * 0.05)(Dc, H, D) * (Dc ** -0.5)),
            "w_o": _w((lambda *s: _rng.normal(s) * 0.05)(H, D, M) * ((H * D) ** -0.5)),
        }
    _A_in = _A_setup()

    def _B_setup():
        B, S, D, F, C = 1, 2048, 1024, 3584, 2
        return {
            "x": _w((lambda *s: _rng.normal(s) * 0.05)(B, S, D)),
            "w_r": _w((lambda *s: _rng.normal(s) * 0.05)(D)),
            "w_gate": _w((lambda *s: _rng.normal(s) * 0.05)(D, F)),
            "w_up": _w((lambda *s: _rng.normal(s) * 0.05)(D, F)),
            "w_down": _w((lambda *s: _rng.normal(s) * 0.05)(F, D)),
        }
    _B_in = _B_setup()

    return {
        "A_x": _A_in["x"],
        "A_c_kv": _A_in["c_kv"],
        "A_w_q": _A_in["w_q"],
        "A_w_uk": _A_in["w_uk"],
        "A_w_uv": _A_in["w_uv"],
        "A_w_o": _A_in["w_o"],
        "B_x": _B_in["x"],
        "B_w_r": _B_in["w_r"],
        "B_w_gate": _B_in["w_gate"],
        "B_w_up": _B_in["w_up"],
        "B_w_down": _B_in["w_down"],
    }

def reference(A_x, A_c_kv, A_w_q, A_w_uk, A_w_uv, A_w_o, B_x, B_w_r, B_w_gate, B_w_up, B_w_down):
    def _A_ref(x, c_kv, w_q, w_uk, w_uv, w_o):
        B, Sq, M = x.shape[0], x.shape[1], x.shape[2]
        Sk = c_kv.shape[1]
        H, D = w_q.shape[1], w_q.shape[2]
        q = jnp.einsum("bqm,mhd->bhqd", x, w_q)
        k = jnp.einsum("bkc,chd->bhkd", c_kv, w_uk)
        v = jnp.einsum("bkc,chd->bhkd", c_kv, w_uv)
        scores = jnp.einsum("bhqd,bhkd->bhqk", q, k) * (D ** -0.5)
        off = Sk - Sq
        qi = jnp.arange(Sq)[:, None]
        kj = jnp.arange(Sk)[None, :]
        cmask = kj <= (qi + off)
        scores = jnp.where(cmask[None, None], scores, -1e9)
        p = _softmax(scores, axis=-1)
        ctx = jnp.einsum("bhqk,bhkd->bhqd", p, v)
        return jnp.einsum("bhqd,hdm->bqm", ctx, w_o)

    def _B_ref(x, w_r, w_gate, w_up, w_down):
        B, S, D = x.shape
        C = 2
        r = x @ w_r
        idx = jnp.argsort(-r, axis=-1)[:, :C]
        idx_e = jnp.repeat(idx.reshape(B, C, 1), D, axis=2)
        x_sel = jnp.take_along_axis(x, idx_e, axis=1)
        g = _silu(x_sel @ w_gate)
        u = x_sel @ w_up
        y = (g * u) @ w_down
        r_sel = _sigmoid(jnp.take_along_axis(r, idx, axis=1))
        y = y * r_sel.reshape(B, C, 1)
        b_off = (jnp.arange(B) * S).reshape(B, 1)
        flat_idx = (idx + b_off).reshape(B * C)
        zero = (x * 0.0).reshape(B * S, D)
        upd = _scatter_add(zero, flat_idx, y.reshape(B * C, D), axis=0)
        return x + upd.reshape(B, S, D)

    x = A_x
    h = x + _A_ref(_layernorm(x, axis=-1), A_c_kv, A_w_q, A_w_uk, A_w_uv, A_w_o)
    h2 = h + _B_ref(_layernorm(h, axis=-1), B_w_r, B_w_gate, B_w_up, B_w_down)
    return h2
```

```python
import math
import os

import jax
import jax.numpy as jnp
from jax import lax
import jax.experimental.pallas as pl
import jax.experimental.pallas.tpu as pltpu

S, M, H, D, DC, F = 2048, 1024, 32, 128, 512, 3584
RB = 256
NB = S // RB
NEG = -1e9 * math.log2(math.e)
QSCALE = (D ** -0.5) * math.log2(math.e)
EPS = 1e-5
BF16, F32 = jnp.bfloat16, jnp.float32


def _cfg(name, default):
    return int(os.environ.get("KCFG_" + name, default))


def _r16(x):
    return x.astype(BF16).astype(F32)


def _layernorm(xf):
    mean = jnp.sum(xf, axis=-1, keepdims=True) * (1.0 / M)
    cen = xf - mean
    var = jnp.sum(cen * cen, axis=-1, keepdims=True) * (1.0 / M)
    den = _r16(jnp.sqrt(_r16(_r16(var) + _r16(jnp.full(var.shape, EPS, F32)))))
    return _r16(xf - _r16(mean)) / den


def _nt(a, b):
    return lax.dot_general(a, b, (((1,), (1,)), ((), ())), preferred_element_type=F32)


def _nn(a, b):
    return jnp.dot(a, b, preferred_element_type=F32)


def _kernel(x_h, ckv_h, wq_h, wuk_h, wuv_h, wo_h, wr_h, wg_h, wu_h, wd_h, out_h,
            x_v, xn_v, ckv_v, wq_v, wuk_v, wuv_v, wo_v, wr_v, wg_v, wu_v, wd_v, ctx_v, out_v,
            wqa, wka, wva, wqb, wkb, wvb,
            qa, ka, va, qb, kb, vb,
            s0, s1, p0, p1, l0, l1, sems, osem):
    copies = [
        pltpu.make_async_copy(x_h, x_v, sems.at[0]),
        pltpu.make_async_copy(ckv_h, ckv_v, sems.at[1]),
        pltpu.make_async_copy(wq_h.bitcast(jnp.uint32), wq_v, sems.at[2]),
        pltpu.make_async_copy(wuk_h.bitcast(jnp.uint32), wuk_v, sems.at[3]),
        pltpu.make_async_copy(wuv_h.bitcast(jnp.uint32), wuv_v, sems.at[4]),
        pltpu.make_async_copy(wo_h, wo_v, sems.at[5]),
        pltpu.make_async_copy(wr_h, wr_v, sems.at[6]),
        pltpu.make_async_copy(wg_h, wg_v, sems.at[7]),
        pltpu.make_async_copy(wu_h, wu_v, sems.at[8]),
        pltpu.make_async_copy(wd_h, wd_v, sems.at[9]),
    ]
    for c in copies:
        c.start()

    copies[0].wait()
    for i in range(NB):
        rows = pl.ds(i * RB, RB)
        xn_v[rows, :] = _layernorm(x_v[rows, :].astype(F32)).astype(BF16)
    for c in copies[1:5]:
        c.wait()

    wq32, wuk32, wuv32 = wq_v, wuk_v, wuv_v

    def unpack(src, dst, pair, hi, nrows):
        for c in range(nrows // 256):
            w = src[pl.ds(pair + c * 256 * (H // 2), 256, stride=H // 2), :]
            w = (w & jnp.uint32(0xFFFF0000)) if hi else (w << 16)
            dst[pl.ds(c * 256, 256), :] = pltpu.bitcast(w, F32).astype(BF16)

    def unpack_head(pair, hi, wq_d, wk_d, wv_d):
        unpack(wq32, wq_d, pair, hi, M)
        unpack(wuk32, wk_d, pair, hi, DC)
        unpack(wuv32, wv_d, pair, hi, DC)

    def proj_q(i, wq_d, q_d):
        rows = pl.ds(i * RB, RB)
        q_d[rows, :] = (_nn(xn_v[rows, :], wq_d[...]) * QSCALE).astype(BF16)

    def proj_kv(i, wk_d, wv_d, k_d, v_d):
        rows = pl.ds(i * RB, RB)
        c = ckv_v[rows, :]
        k_d[rows, :] = _nn(c, wk_d[...]).astype(BF16)
        v_d[rows, :] = _nn(c, wv_d[...]).astype(BF16)

    def stage_a(i, q_r, k_r, s_r):
        rr = lax.broadcasted_iota(jnp.int32, (128, 128), 0)
        cc = lax.broadcasted_iota(jnp.int32, (128, 128), 1)
        tri = cc <= rr
        q = q_r[pl.ds(i * RB, RB), :]
        cw = _cfg("ACW", 256)
        full = 2 * i * 128
        for c0 in range(0, full, cw):
            s_r[:, pl.ds(c0, cw)] = _nt(q, k_r[pl.ds(c0, cw), :])
        s = _nt(q, k_r[pl.ds(full, 128), :])
        s_r[pl.ds(0, 128), pl.ds(full, 128)] = jnp.where(tri, s[:128], NEG)
        s_r[pl.ds(128, 128), pl.ds(full, 128)] = s[128:]
        s = _nt(q[128:], k_r[pl.ds(full + 128, 128), :])
        s_r[pl.ds(128, 128), pl.ds(full + 128, 128)] = jnp.where(tri, s, NEG)

    def stage_b(i, s_r, p_r, l_r):
        g = _cfg("BG", 64)
        for r0 in range(0, RB, g):
            rows = pl.ds(r0, g)
            nt = 2 * i + 1 + (r0 >= 128)
            m = s_r[rows, pl.ds(0, 128)]
            for t in range(1, nt):
                m = jnp.maximum(m, s_r[rows, pl.ds(t * 128, 128)])
            m = jnp.max(m, axis=-1, keepdims=True)
            l = None
            for t in range(nt):
                p = jnp.exp2(s_r[rows, pl.ds(t * 128, 128)] - m)
                l = p if l is None else l + p
                p_r[rows, pl.ds(t * 128, 128)] = p.astype(BF16)
            l_r[rows, :] = jnp.broadcast_to(jnp.sum(l, axis=-1, keepdims=True), (g, 128))

    def stage_c(i, v_r, p_r, l_r, head):
        w = (2 * i + 1) * 128
        acc = _nn(p_r[:, pl.ds(0, w)], v_r[pl.ds(0, w), :])
        low = _nn(p_r[pl.ds(128, 128), pl.ds(w, 128)], v_r[pl.ds(w, 128), :])
        inv = 1.0 / l_r[...]
        cols = pl.ds(pl.multiple_of(head * D, D), D)
        ctx_v[pl.ds(i * RB, 128), cols] = (acc[:128] * inv[:128]).astype(BF16)
        ctx_v[pl.ds(i * RB + 128, 128), cols] = ((acc[128:] + low) * inv[128:]).astype(BF16)

    sbuf, pbuf, lbuf = (s0, s1), (p0, p1), (l0, l1)
    bufa, bufb = (qa, ka, va), (qb, kb, vb)
    wa, wb = (wqa, wka, wva), (wqb, wkb, wvb)

    def attention(cur, head, filler):
        q_r, k_r, v_r = cur
        for t in range(NB + 2):
            if t < NB:
                stage_a(t, q_r, k_r, sbuf[t % 2])
            if 1 <= t <= NB:
                stage_b(t - 1, sbuf[(t - 1) % 2], pbuf[(t - 1) % 2], lbuf[(t - 1) % 2])
            if t < NB and filler is not None:
                filler(t)
            if t >= 2:
                stage_c(t - 2, v_r, pbuf[t % 2], lbuf[t % 2], head)

    def projector(w, buf):
        def f(t):
            proj_q(t, w[0], buf[0])
            proj_kv(t, w[1], w[2], buf[1], buf[2])
        return f

    unpack_head(0, False, *wa)
    for i in range(NB):
        projector(wa, bufa)(i)

    def pair_body(j, carry):
        unpack_head(j, True, *wb)
        attention(bufa, 2 * j, projector(wb, bufb))
        unpack_head(j + 1, False, *wa)
        attention(bufb, 2 * j + 1, projector(wa, bufa))
        return carry

    lax.fori_loop(0, H // 2 - 1, pair_body, 0)
    unpack_head(H // 2 - 1, True, *wb)
    attention(bufa, H - 2, projector(wb, bufb))
    for c in copies[5:]:
        c.wait()
    attention(bufb, H - 1, None)

    wr = wr_v[...].astype(F32).reshape(1, M)
    best = []
    for i in range(NB):
        rows = pl.ds(i * RB, RB)
        attn = _r16(_nn(ctx_v[rows, :], wo_v[...]))
        h = _r16(x_v[rows, :].astype(F32) + attn)
        hn = _r16(_layernorm(h))
        x_v[rows, :] = h.astype(BF16)
        xn_v[rows, :] = hn.astype(BF16)
        out_v[rows, :] = (h + hn).astype(BF16)
        pltpu.make_async_copy(out_v.at[rows, :], out_h.at[rows, :], sems.at[i]).start()
        best.append(_r16(jnp.sum(hn * wr, axis=-1, keepdims=True)))

    r = jnp.concatenate(best, axis=0)
    ridx = lax.broadcasted_iota(jnp.int32, (S, 1), 0)
    r1 = jnp.max(r, axis=0, keepdims=True)
    i1 = jnp.min(jnp.where(r == r1, ridx, S), axis=0, keepdims=True)
    rr = jnp.where(ridx == i1, -jnp.inf, r)
    r2 = jnp.max(rr, axis=0, keepdims=True)
    i2 = jnp.min(jnp.where(rr == r2, ridx, S), axis=0, keepdims=True)
    idx1, idx2 = i1[0, 0], i2[0, 0]

    row16 = lax.broadcasted_iota(jnp.int32, (16, M), 0)
    g1 = pl.multiple_of((idx1 // 16) * 16, 16)
    g2 = pl.multiple_of((idx2 // 16) * 16, 16)
    hn1 = xn_v[pl.ds(g1, 16), :].astype(F32)
    hn2 = xn_v[pl.ds(g2, 16), :].astype(F32)
    m1, m2 = row16 == idx1 - g1, row16 == idx2 - g2
    x1 = jnp.sum(jnp.where(m1, hn1, 0.0), axis=0, keepdims=True)
    x2 = jnp.sum(jnp.where(m2, hn2, 0.0), axis=0, keepdims=True)
    xs = jnp.where(row16 == 0, x1, jnp.where(row16 == 1, x2, 0.0)).astype(BF16)

    gate = _r16(_nn(xs, wg_v[...]))
    up = _r16(_nn(xs, wu_v[...]))
    act = _r16(_r16(gate * _r16(jax.nn.sigmoid(gate))) * up).astype(BF16)
    y = _r16(_nn(act, wd_v[...]))
    y1 = _r16(y[0:1] * _r16(jax.nn.sigmoid(r1)))
    y2 = _r16(y[1:2] * _r16(jax.nn.sigmoid(r2)))

    for i in range(NB):
        rows = pl.ds(i * RB, RB)
        pltpu.make_async_copy(out_v.at[rows, :], out_h.at[rows, :], sems.at[i]).wait()

    def fix(g, mask, hn, yrow):
        h = x_v[pl.ds(g, 16), :].astype(F32)
        old = out_v[pl.ds(g, 16), :]
        new = (h + _r16(hn + yrow)).astype(BF16)
        out_v[pl.ds(g, 16), :] = jnp.where(mask, new, old)

    fix(g1, m1, hn1, y1)
    fix(g2, m2, hn2, y2)
    c1 = pltpu.make_async_copy(out_v.at[pl.ds(g1, 16), :], out_h.at[pl.ds(g1, 16), :], osem.at[0])
    c1.start()

    @pl.when(g1 != g2)
    def _():
        c2 = pltpu.make_async_copy(out_v.at[pl.ds(g2, 16), :], out_h.at[pl.ds(g2, 16), :], osem.at[1])
        c2.start()
        c2.wait()

    c1.wait()


@jax.jit
def pallas_sequential_preLN__compressed_kv_cla__moe_arch_mod__prompt_kernel(
    A_x: jax.Array,
    A_c_kv: jax.Array,
    A_w_q: jax.Array,
    A_w_uk: jax.Array,
    A_w_uv: jax.Array,
    A_w_o: jax.Array,
    B_x: jax.Array,
    B_w_r: jax.Array,
    B_w_gate: jax.Array,
    B_w_up: jax.Array,
    B_w_down: jax.Array,
):
    del B_x
    hbm = pl.BlockSpec(memory_space=pl.ANY)
    vm = pltpu.VMEM
    scratch = [
        vm((S, M), BF16), vm((S, M), BF16), vm((S, DC), BF16),
        vm((M * H // 2, D), jnp.uint32), vm((DC * H // 2, D), jnp.uint32), vm((DC * H // 2, D), jnp.uint32),
        vm((H * D, M), BF16), vm((M,), BF16), vm((M, F), BF16), vm((M, F), BF16), vm((F, M), BF16),
        vm((S, H * D), BF16), vm((S, M), BF16),
        vm((M, D), BF16), vm((DC, D), BF16), vm((DC, D), BF16),
        vm((M, D), BF16), vm((DC, D), BF16), vm((DC, D), BF16),
        vm((S, D), BF16), vm((S, D), BF16), vm((S, D), BF16),
        vm((S, D), BF16), vm((S, D), BF16), vm((S, D), BF16),
        vm((RB, S), F32), vm((RB, S), F32), vm((RB, S), BF16), vm((RB, S), BF16),
        vm((RB, 128), F32), vm((RB, 128), F32),
        pltpu.SemaphoreType.DMA((10,)), pltpu.SemaphoreType.DMA((2,)),
    ]
    out = pl.pallas_call(
        _kernel,
        out_shape=jax.ShapeDtypeStruct((S, M), BF16),
        in_specs=[hbm] * 10,
        out_specs=hbm,
        scratch_shapes=scratch,
        compiler_params=pltpu.CompilerParams(vmem_limit_bytes=110 * 1024 * 1024),
    )(
        A_x.reshape(S, M), A_c_kv.reshape(S, DC),
        A_w_q.reshape(M * H, D), A_w_uk.reshape(DC * H, D), A_w_uv.reshape(DC * H, D),
        A_w_o.reshape(H * D, M), B_w_r, B_w_gate, B_w_up, B_w_down,
    )
    return out.reshape(1, S, M)
```

```python
import functools
import math
import os

import jax
import jax.numpy as jnp
from jax import lax
import jax.experimental.pallas as pl
import jax.experimental.pallas.tpu as pltpu

S, M, H, D, DC, F = 2048, 1024, 32, 128, 512, 3584
RB = 256
NB = S // RB
NEG = -1e9 * math.log2(math.e)
QSCALE = (D ** -0.5) * math.log2(math.e)
EPS = 1e-5
BF16, F32 = jnp.bfloat16, jnp.float32


def _cfg(name, default):
    return int(os.environ.get("KCFG_" + name, default))


def _flags():
    fl = {}
    for kv in os.environ.get("KCFG_FLAGS", "").split(","):
        if kv:
            k, v = kv.split(":")
            fl[k] = {"T": True, "F": False}.get(v, v)
            if isinstance(fl[k], str):
                fl[k] = int(v)
    return fl or None


def _scope(name):
    import contextlib
    return jax.named_scope(name) if _cfg("SCOPE", 0) else contextlib.nullcontext()


def _r16(x):
    return x.astype(BF16).astype(F32)


def _layernorm(xf):
    mean = jnp.sum(xf, axis=-1, keepdims=True) * (1.0 / M)
    cen = xf - mean
    var = jnp.sum(cen * cen, axis=-1, keepdims=True) * (1.0 / M)
    den = _r16(jnp.sqrt(_r16(_r16(var) + _r16(jnp.full(var.shape, EPS, F32)))))
    return _r16(xf - _r16(mean)) / den


def _pk(x):
    if _cfg("PK16", 0) and x.shape[0] > 16:
        return jnp.concatenate([_pk(x[r:r + 16]) for r in range(0, x.shape[0], 16)], axis=0)
    return pltpu.bitcast(x.astype(BF16), jnp.uint32)


def _up(w):
    return pltpu.bitcast(w, BF16)


def _nt(a, b):
    return lax.dot_general(a, b, (((1,), (1,)), ((), ())), preferred_element_type=F32)


def _nn(a, b):
    return jnp.dot(a, b, preferred_element_type=F32)


def _kernel(x_h, ckv_h, wq_h, wuk_h, wuv_h, wo_h, wr_h, wg_h, wu_h, wd_h, out_h,
            x_v, xn_v, ckv_v, ckp_v, wq_v, wuk_v, wuv_v, wo_v, wop_v, wr_v, wg_v, wu_v, wd_v, ctx_v, out_v,
            wqa, wka, wva, wqb, wkb, wvb,
            qa, ka, va, qb, kb, vb,
            s0, s1, s2, p0, p1, p2, p3, l0, l1, l2, l3, zero_s, sems, osem):
    zero_s[0] = 0
    zero_s[1] = 0
    def cp(src, dst, k):
        return pltpu.make_async_copy(src, dst, sems.at[k])

    def halves(w_h, w_v, k):
        w32 = w_h.bitcast(jnp.uint32)
        return [cp(w32.at[:, hf], w_v.at[hf], k + hf) for hf in range(2)]

    c_wq, c_wuk, c_wuv = halves(wq_h, wq_v, 2), halves(wuk_h, wuk_v, 4), halves(wuv_h, wuv_v, 6)
    c_ckv, c_x = cp(ckv_h, ckv_v, 0), cp(x_h, x_v, 1)
    late = [cp(wo_h, wo_v, 8), cp(wr_h, wr_v, 9), cp(wg_h, wg_v, 10), cp(wu_h, wu_v, 11), cp(wd_h, wd_v, 12)]
    second = [c_wq[1], c_wuk[1], c_wuv[1]]
    for c in [c_ckv, c_wuk[0], c_wuv[0], c_x, c_wq[0]] + second + late:
        c.start()

    wq32 = wq_v.reshape(2 * M * 8, D)
    wuk32 = wuk_v.reshape(2 * DC * 8, D)
    wuv32 = wuv_v.reshape(2 * DC * 8, D)

    def unpack(src, dst, pair, hi, nrows):
        base = (pair // 8) * (nrows * 8) + pair % 8
        for c in range(nrows // 256):
            w = src[pl.ds(base + c * 256 * 8, 256, stride=8), :]
            w = (w & jnp.uint32(0xFFFF0000)) if hi else (w << 16)
            dst[pl.ds(c * 128, 128), :] = _pk(pltpu.bitcast(w, F32))

    def unpack_head(pair, hi, wq_d, wk_d, wv_d):
        unpack(wq32, wq_d, pair, hi, M)
        unpack(wuk32, wk_d, pair, hi, DC)
        unpack(wuv32, wv_d, pair, hi, DC)

    PM = _cfg("PM", 256)

    def tied(w_r, tok):
        w = w_r[...]
        if tok is not None:
            parts = []
            for r0 in range(0, w.shape[0], 64):
                parts += [w[r0:r0 + 8] | tok, w[r0 + 8:r0 + 64]]
            w = jnp.concatenate(parts, axis=0)
        return _up(w)

    def proj(i, w, buf, toks):
        toks = toks or [None] * 4
        for half in range(RB // PM):
            rows = pl.ds((i * RB + half * PM) // 2, PM // 2)
            buf[0][rows, :] = _pk(_nn(_up(xn_v[rows, :]), tied(w[0], toks[2 * half])) * QSCALE)
            buf[1][rows, :] = _pk(_nn(_up(ckp_v[rows, :]), tied(w[1], toks[2 * half + 1])))
            buf[2][rows, :] = _pk(_nn(_up(ckp_v[rows, :]), tied(w[2], toks[2 * half + 1])))

    def stage_a(i, q_r, k_r, s_r):
        rr = lax.broadcasted_iota(jnp.int32, (128, 128), 0)
        cc = lax.broadcasted_iota(jnp.int32, (128, 128), 1)
        tri = cc <= rr
        q = _up(q_r[pl.ds(i * RB // 2, RB // 2), :])
        cw = _cfg("ACW", 256)
        full = 2 * i * 128
        for c0 in range(0, full, cw):
            s_r[:, pl.ds(c0, cw)] = (_nt(q, _up(k_r[pl.ds(c0 // 2, cw // 2), :])))
        s = _nt(q, _up(k_r[pl.ds(full // 2, 64), :]))
        s_r[pl.ds(0, 128), pl.ds(full, 128)] = (jnp.where(tri, s[:128], NEG))
        s_r[pl.ds(128, 128), pl.ds(full, 128)] = (s[128:])
        s = _nt(q[128:], _up(k_r[pl.ds(full // 2 + 64, 64), :]))
        s_r[pl.ds(128, 128), pl.ds(full + 128, 128)] = (jnp.where(tri, s, NEG))

    def stage_b(i, s_r, p_r, l_r):
        g = _cfg("BG", 16)
        z = zero_s[0]
        dep = _cfg("DEP", 0)
        zvec = jnp.full((g // 2, 128), z, jnp.int32).astype(jnp.uint32)
        toks = []
        chain, lag, sett = [], _cfg("LAG", 2), _cfg("SET", 2)
        zvg = jnp.full((g, 128), z, jnp.int32).astype(jnp.uint32)
        for r0 in range(0, RB, g):
            rows = pl.ds(r0, g)
            rows1 = pl.ds(pl.multiple_of(r0 + z, 8), g) if _cfg("OPAQUE", 0) else rows
            nt = 2 * i + 1 + (r0 >= 128)
            m = s_r[rows1, pl.ds(0, 128)]
            for t in range(1, nt):
                m = jnp.maximum(m, s_r[rows1, pl.ds(t * 128, 128)])
            if r0 % (RB // 4) == _cfg("TOKG", 0) * g:
                toks.append(pltpu.bitcast(m[:8], jnp.uint32) & zvec[:8])
            m = jnp.max(m, axis=-1, keepdims=True)
            l = None
            mb = jnp.broadcast_to(m, (g, 128))
            for t in range(nt):
                if lag and t % sett == 0 and len(chain) >= lag:
                    mt = mb + chain.pop(0)
                elif t == 0:
                    mt = mb
                p = jnp.exp2(s_r[rows, pl.ds(t * 128, 128)] - mt)
                l = p if l is None else l + p
                if lag and (t % sett == sett - 1 or t == nt - 1):
                    chain.append(pltpu.bitcast(pltpu.bitcast(l, jnp.uint32) & zvg, F32))
                pw = _pk(p)
                if dep and t % dep == dep - 1:
                    pw = pw | (pltpu.bitcast(l[: g // 2] + l[g // 2:], jnp.uint32) & zvec)
                p_r[pl.ds(r0 // 2, g // 2), pl.ds(t * 128, 128)] = pw
            l_r[rows, :] = jnp.broadcast_to(jnp.sum(l, axis=-1, keepdims=True), (g, 128))
        return toks if _cfg("TOK", 0) else None

    def stage_c(i, v_r, p_r, l_r, head):
        cols = pl.ds(pl.multiple_of(head * D, D), D)
        if _cfg("CM", 128) == 256:
            w = (2 * i + 1) * 128
            acc = _nn(_up(p_r[:, pl.ds(0, w)]), _up(v_r[pl.ds(0, w // 2), :]))
            low = _nn(_up(p_r[pl.ds(64, 64), pl.ds(w, 128)]), _up(v_r[pl.ds(w // 2, 64), :]))
            inv = 1.0 / l_r[...]
            ctx_v[pl.ds(i * RB // 2, 64), cols] = _pk(acc[:128] * inv[:128])
            ctx_v[pl.ds(i * RB // 2 + 64, 64), cols] = _pk((acc[128:] + low) * inv[128:])
            return
        for half in range(2):
            w = (2 * i + 1 + half) * 128
            acc = _nn(_up(p_r[pl.ds(half * 64, 64), pl.ds(0, w)]), _up(v_r[pl.ds(0, w // 2), :]))
            inv = 1.0 / l_r[pl.ds(half * 128, 128), :]
            ctx_v[pl.ds(i * RB // 2 + half * 64, 64), cols] = _pk(acc * inv)
        if _cfg("TOKC", 0):
            return pltpu.bitcast(acc[:8], jnp.uint32) & jnp.full((8, 128), zero_s[0], jnp.int32).astype(jnp.uint32)

    NS, NP = _cfg("NS", 3), _cfg("NP", 3)
    sbuf, pbuf, lbuf = (s0, s1, s2), (p0, p1, p2, p3), (l0, l1, l2, l3)
    bufa, bufb = (qa, ka, va), (qb, kb, vb)
    wa, wb = (wqa, wka, wva), (wqb, wkb, wvb)

    def projector(w, buf):
        return lambda i, toks=None: proj(i, w, buf, toks)

    def head_pair(head, fill, unpack_a, unpack_b):
        tasks = [(bufa, head, i) for i in range(NB)] + [(bufb, head + 1, i) for i in reversed(range(NB))]
        n = len(tasks)
        ctok = None
        for t in range(max([n + 1] + list(fill)) + 1):
            for f in fill.get(t, ()):
                f([ctok] * 4 if ctok is not None else None)
            if t == 1 and unpack_a is not None:
                unpack_a()
            if t == NB + 1 and unpack_b is not None:
                unpack_b()
            if t < n:
                (q_r, k_r, _), _, i = tasks[t]
                stage_a(i, q_r, k_r, sbuf[t % NS])
            if 1 <= t <= n:
                toks = stage_b(tasks[t - 1][2], sbuf[(t - 1) % NS], pbuf[(t - 1) % NP], lbuf[(t - 1) % NP])
            if 2 <= t < n + 2:
                (_, _, v_r), hd, i = tasks[t - 2]
                ctok = stage_c(i, v_r, pbuf[(t - 2) % NP], lbuf[(t - 2) % NP], hd)

    def fills(first, second):
        fill = {0: [functools.partial(first, 0), functools.partial(first, 1)]}
        for i in range(2, NB):
            fill[i - 1] = [functools.partial(first, i)]
        if second is not None:
            for i in range(NB):
                fill[NB - 1 + _cfg("F2", 3) + i] = fill.get(NB - 1 + _cfg("F2", 3) + i, []) + [functools.partial(second, i)]
        return fill

    with _scope("kv0"):
        c_ckv.wait()
        for i in range(NB):
            ckp_v[pl.ds(i * RB // 2, RB // 2), :] = _pk(ckv_v[pl.ds(i * RB, RB), :])
        c_wuk[0].wait()
        unpack(wuk32, wka, 0, False, DC)
        unpack(wuk32, wkb, 0, True, DC)
        for i in range(NB):
            rows = pl.ds(i * RB // 2, RB // 2)
            ka[rows, :] = _pk(_nn(_up(ckp_v[rows, :]), _up(wka[...])))
        c_wuv[0].wait()
        unpack(wuv32, wva, 0, False, DC)
        unpack(wuv32, wvb, 0, True, DC)
        for i in range(NB):
            rows = pl.ds(i * RB // 2, RB // 2)
            va[rows, :] = _pk(_nn(_up(ckp_v[rows, :]), _up(wva[...])))
    with _scope("ln1"):
        c_x.wait()
        for i in range(NB):
            xn_v[pl.ds(i * RB // 2, RB // 2), :] = _pk(_layernorm(x_v[pl.ds(i * RB, RB), :].astype(F32)))
    with _scope("q0"):
        c_wq[0].wait()
        unpack(wq32, wqa, 0, False, M)
        unpack(wq32, wqb, 0, True, M)
        for i in range(NB):
            rows = pl.ds(i * RB // 2, RB // 2)
            qa[rows, :] = _pk(_nn(_up(xn_v[rows, :]), _up(wqa[...])) * QSCALE)

    def pair_body(j, carry):
        @pl.when(j == H // 4 - 1)
        def _():
            for c in second:
                c.wait()

        head_pair(2 * j, fills(projector(wb, bufb), projector(wa, bufa)),
                  lambda: unpack_head(j + 1, False, *wa), lambda: unpack_head(j + 1, True, *wb))
        return carry

    with _scope("loop"):
        lax.fori_loop(0, H // 2 - 1, pair_body, 0)
    if _cfg("LOOPONLY", 0):
        for c in late:
            c.wait()
        out_v[...] = _up(ctx_v[:, pl.ds(0, M)])
        c = pltpu.make_async_copy(out_v, out_h, osem.at[0])
        c.start()
        c.wait()
        return
    for c in late:
        c.wait()
    wr = wr_v[...].astype(F32).reshape(1, M)
    best = {}

    def out_block(i, toks=None):
        OM = _cfg("OM", 128)
        for r0 in range(i * RB, (i + 1) * RB, OM):
            rows, rows2 = pl.ds(r0, OM), pl.ds(r0 // 2, OM // 2)
            attn = _r16(_nn(_up(ctx_v[rows2, :]), _up(wop_v[...])))
            h = _r16(x_v[rows, :].astype(F32) + attn)
            hn = _r16(_layernorm(h))
            x_v[rows, :] = h.astype(BF16)
            xn_v[rows2, :] = _pk(hn)
            out_v[rows, :] = (h + hn).astype(BF16)
            best[r0] = _r16(jnp.sum(hn * wr, axis=-1, keepdims=True))
        rows = pl.ds(i * RB, RB)
        pltpu.make_async_copy(out_v.at[rows, :], out_h.at[rows, :], sems.at[i]).start()

    def pack_wo():
        for c in range(H * D // 256):
            wop_v[pl.ds(c * 128, 128), :] = _pk(wo_v[pl.ds(c * 256, 256), :])

    with _scope("last"):
        fill = fills(projector(wb, bufb), None)
        for u in range(NB):
            fill[NB + 3 + u] = [functools.partial(out_block, NB - 1 - u)]
        head_pair(H - 2, fill, pack_wo, None)
    sc = _scope("tail")
    sc.__enter__()
    best = [best[k] for k in sorted(best)]
    r = jnp.concatenate(best, axis=0)
    ridx = lax.broadcasted_iota(jnp.int32, (S, 1), 0)
    r1 = jnp.max(r, axis=0, keepdims=True)
    i1 = jnp.min(jnp.where(r == r1, ridx, S), axis=0, keepdims=True)
    rr = jnp.where(ridx == i1, -jnp.inf, r)
    r2 = jnp.max(rr, axis=0, keepdims=True)
    i2 = jnp.min(jnp.where(rr == r2, ridx, S), axis=0, keepdims=True)
    idx1, idx2 = i1[0, 0], i2[0, 0]

    row16 = lax.broadcasted_iota(jnp.int32, (16, M), 0)
    g1 = pl.multiple_of((idx1 // 16) * 16, 16)
    g2 = pl.multiple_of((idx2 // 16) * 16, 16)
    hn1 = _up(xn_v[pl.ds(pl.multiple_of(g1 // 2, 8), 8), :]).astype(F32)
    hn2 = _up(xn_v[pl.ds(pl.multiple_of(g2 // 2, 8), 8), :]).astype(F32)
    m1, m2 = row16 == idx1 - g1, row16 == idx2 - g2
    x1 = jnp.sum(jnp.where(m1, hn1, 0.0), axis=0, keepdims=True)
    x2 = jnp.sum(jnp.where(m2, hn2, 0.0), axis=0, keepdims=True)
    xs = jnp.where(row16 == 0, x1, jnp.where(row16 == 1, x2, 0.0)).astype(BF16)

    gate = _r16(_nn(xs, wg_v[...]))
    up = _r16(_nn(xs, wu_v[...]))
    act = _r16(_r16(gate * _r16(jax.nn.sigmoid(gate))) * up).astype(BF16)
    y = _r16(_nn(act, wd_v[...]))
    y1 = _r16(y[0:1] * _r16(jax.nn.sigmoid(r1)))
    y2 = _r16(y[1:2] * _r16(jax.nn.sigmoid(r2)))

    for i in range(NB):
        rows = pl.ds(i * RB, RB)
        pltpu.make_async_copy(out_v.at[rows, :], out_h.at[rows, :], sems.at[i]).wait()

    def fix(g, mask, hn, yrow):
        h = x_v[pl.ds(g, 16), :].astype(F32)
        old = out_v[pl.ds(g, 16), :]
        new = (h + _r16(hn + yrow)).astype(BF16)
        out_v[pl.ds(g, 16), :] = jnp.where(mask, new, old)

    fix(g1, m1, hn1, y1)
    fix(g2, m2, hn2, y2)
    c1 = pltpu.make_async_copy(out_v.at[pl.ds(g1, 16), :], out_h.at[pl.ds(g1, 16), :], osem.at[0])
    c1.start()

    @pl.when(g1 != g2)
    def _():
        c2 = pltpu.make_async_copy(out_v.at[pl.ds(g2, 16), :], out_h.at[pl.ds(g2, 16), :], osem.at[1])
        c2.start()
        c2.wait()

    c1.wait()
    sc.__exit__(None, None, None)


@jax.jit
def pallas_sequential_preLN__compressed_kv_cla__moe_arch_mod__prompt_kernel(
    A_x: jax.Array,
    A_c_kv: jax.Array,
    A_w_q: jax.Array,
    A_w_uk: jax.Array,
    A_w_uv: jax.Array,
    A_w_o: jax.Array,
    B_x: jax.Array,
    B_w_r: jax.Array,
    B_w_gate: jax.Array,
    B_w_up: jax.Array,
    B_w_down: jax.Array,
):
    del B_x
    hbm = pl.BlockSpec(memory_space=pl.ANY)
    vm = pltpu.VMEM
    u32 = jnp.uint32
    scratch = [
        vm((S, M), BF16), vm((S // 2, M), u32), vm((S, DC), BF16), vm((S // 2, DC), u32),
        vm((2, M, 8, D), u32), vm((2, DC, 8, D), u32), vm((2, DC, 8, D), u32),
        vm((H * D, M), BF16), vm((H * D // 2, M), u32), vm((M,), BF16), vm((M, F), BF16), vm((M, F), BF16), vm((F, M), BF16),
        vm((S // 2, H * D), u32), vm((S, M), BF16),
        vm((M // 2, D), u32), vm((DC // 2, D), u32), vm((DC // 2, D), u32),
        vm((M // 2, D), u32), vm((DC // 2, D), u32), vm((DC // 2, D), u32),
        vm((S // 2, D), u32), vm((S // 2, D), u32), vm((S // 2, D), u32),
        vm((S // 2, D), u32), vm((S // 2, D), u32), vm((S // 2, D), u32),
        vm((RB, S), F32), vm((RB, S), F32), vm((RB, S), F32),
        vm((RB // 2, S), u32), vm((RB // 2, S), u32), vm((RB // 2, S), u32), vm((RB // 2, S), u32),
        vm((RB, 128), F32), vm((RB, 128), F32), vm((RB, 128), F32), vm((RB, 128), F32),
        pltpu.SMEM((2,), jnp.int32),
        pltpu.SemaphoreType.DMA((13,)), pltpu.SemaphoreType.DMA((2,)),
    ]
    out = pl.pallas_call(
        _kernel,
        out_shape=jax.ShapeDtypeStruct((S, M), BF16),
        in_specs=[hbm] * 10,
        out_specs=hbm,
        scratch_shapes=scratch,
        compiler_params=pltpu.CompilerParams(vmem_limit_bytes=126 * 1024 * 1024, flags=_flags()),
    )(
        A_x.reshape(S, M), A_c_kv.reshape(S, DC),
        A_w_q.reshape(M, 2, H // 2, D), A_w_uk.reshape(DC, 2, H // 2, D), A_w_uv.reshape(DC, 2, H // 2, D),
        A_w_o.reshape(H * D, M), B_w_r, B_w_gate, B_w_up, B_w_down,
    )
    return out.reshape(1, S, M)
```

```python
import functools
import math

import jax
import jax.numpy as jnp
from jax import lax
import jax.experimental.pallas as pl
import jax.experimental.pallas.tpu as pltpu

S, M, H, D, DC, F = 2048, 1024, 32, 128, 512, 3584
RB = 256
NB = S // RB
NEG = -1e9 * math.log2(math.e)
QSCALE = (D ** -0.5) * math.log2(math.e)
EPS = 1e-5
BF16, F32 = jnp.bfloat16, jnp.float32


def _r16(x):
    return x.astype(BF16).astype(F32)


def _layernorm(xf):
    mean = jnp.sum(xf, axis=-1, keepdims=True) * (1.0 / M)
    cen = xf - mean
    var = jnp.sum(cen * cen, axis=-1, keepdims=True) * (1.0 / M)
    den = _r16(jnp.sqrt(_r16(_r16(var) + _r16(jnp.full(var.shape, EPS, F32)))))
    return _r16(xf - _r16(mean)) / den


def _pk(x):
    return pltpu.bitcast(x.astype(BF16), jnp.uint32)


def _up(w):
    return pltpu.bitcast(w, BF16)


def _nt(a, b):
    return lax.dot_general(a, b, (((1,), (1,)), ((), ())), preferred_element_type=F32)


def _nn(a, b):
    return jnp.dot(a, b, preferred_element_type=F32)


def _kernel(x_h, ckv_h, wq_h, wuk_h, wuv_h, wo_h, wr_h, wg_h, wu_h, wd_h, out_h,
            x_v, xn_v, ckv_v, ckp_v, wq_v, wuk_v, wuv_v, wo_v, wop_v, wr_v, wg_v, wu_v, wd_v, ctx_v, out_v,
            wqa, wka, wva, wqb, wkb, wvb,
            qa, ka, va, qb, kb, vb,
            s0, s1, s2, p0, p1, p2, l0, l1, l2, zero_s, sems, osem):
    zero_s[0] = 0
    def cp(src, dst, k):
        return pltpu.make_async_copy(src, dst, sems.at[k])

    def halves(w_h, w_v, k):
        w32 = w_h.bitcast(jnp.uint32)
        return [cp(w32.at[:, hf], w_v.at[hf], k + hf) for hf in range(2)]

    c_wq, c_wuk, c_wuv = halves(wq_h, wq_v, 2), halves(wuk_h, wuk_v, 4), halves(wuv_h, wuv_v, 6)
    c_ckv, c_x = cp(ckv_h, ckv_v, 0), cp(x_h, x_v, 1)
    late = [cp(wo_h, wo_v, 8), cp(wr_h, wr_v, 9), cp(wg_h, wg_v, 10), cp(wu_h, wu_v, 11), cp(wd_h, wd_v, 12)]
    second = [c_wq[1], c_wuk[1], c_wuv[1]]
    for c in [c_x, c_wq[0], c_ckv, c_wuk[0], c_wuv[0]] + second + late:
        c.start()

    wq32 = wq_v.reshape(2 * M * 8, D)
    wuk32 = wuk_v.reshape(2 * DC * 8, D)
    wuv32 = wuv_v.reshape(2 * DC * 8, D)

    def unpack(src, dst, pair, hi, nrows):
        base = (pair // 8) * (nrows * 8) + pair % 8
        for c in range(nrows // 256):
            w = src[pl.ds(base + c * 256 * 8, 256, stride=8), :]
            w = (w & jnp.uint32(0xFFFF0000)) if hi else (w << 16)
            dst[pl.ds(c * 128, 128), :] = _pk(pltpu.bitcast(w, F32))

    def unpack_head(pair, hi, wq_d, wk_d, wv_d):
        unpack(wq32, wq_d, pair, hi, M)
        unpack(wuk32, wk_d, pair, hi, DC)
        unpack(wuv32, wv_d, pair, hi, DC)

    def proj(i, w, buf):
        rows = pl.ds(i * RB // 2, RB // 2)
        buf[0][rows, :] = _pk(_nn(_up(xn_v[rows, :]), _up(w[0][...])) * QSCALE)
        buf[1][rows, :] = _pk(_nn(_up(ckp_v[rows, :]), _up(w[1][...])))
        buf[2][rows, :] = _pk(_nn(_up(ckp_v[rows, :]), _up(w[2][...])))

    def stage_a(i, q_r, k_r, s_r):
        rr = lax.broadcasted_iota(jnp.int32, (128, 128), 0)
        cc = lax.broadcasted_iota(jnp.int32, (128, 128), 1)
        tri = cc <= rr
        q = _up(q_r[pl.ds(i * RB // 2, RB // 2), :])
        cw = 256
        full = 2 * i * 128
        for c0 in range(0, full, cw):
            s_r[:, pl.ds(c0, cw)] = (_nt(q, _up(k_r[pl.ds(c0 // 2, cw // 2), :])))
        s = _nt(q, _up(k_r[pl.ds(full // 2, 64), :]))
        s_r[pl.ds(0, 128), pl.ds(full, 128)] = (jnp.where(tri, s[:128], NEG))
        s_r[pl.ds(128, 128), pl.ds(full, 128)] = (s[128:])
        s = _nt(q[128:], _up(k_r[pl.ds(full // 2 + 64, 64), :]))
        s_r[pl.ds(128, 128), pl.ds(full + 128, 128)] = (jnp.where(tri, s, NEG))

    def stage_b(i, s_r, p_r, l_r):
        g, lag, span = 16, 2, 3
        zero = jnp.full((g, 128), zero_s[0], jnp.int32).astype(jnp.uint32)
        pace = []
        for r0 in range(0, RB, g):
            rows = pl.ds(r0, g)
            nt = 2 * i + 1 + (r0 >= 128)
            m = s_r[rows, pl.ds(0, 128)]
            for t in range(1, nt):
                m = jnp.maximum(m, s_r[rows, pl.ds(t * 128, 128)])
            mb = jnp.broadcast_to(jnp.max(m, axis=-1, keepdims=True), (g, 128))
            l = None
            for t in range(nt):
                if t % span == 0 and len(pace) >= lag:
                    mt = mb + pace.pop(0)
                elif t == 0:
                    mt = mb
                p = jnp.exp2(s_r[rows, pl.ds(t * 128, 128)] - mt)
                l = p if l is None else l + p
                if t % span == span - 1 or t == nt - 1:
                    pace.append(pltpu.bitcast(pltpu.bitcast(l, jnp.uint32) & zero, F32))
                p_r[pl.ds(r0 // 2, g // 2), pl.ds(t * 128, 128)] = _pk(p)
            l_r[rows, :] = jnp.broadcast_to(jnp.sum(l, axis=-1, keepdims=True), (g, 128))

    def stage_c(i, v_r, p_r, l_r, head):
        cols = pl.ds(pl.multiple_of(head * D, D), D)
        for half in range(2):
            w = (2 * i + 1 + half) * 128
            acc = _nn(_up(p_r[pl.ds(half * 64, 64), pl.ds(0, w)]), _up(v_r[pl.ds(0, w // 2), :]))
            inv = 1.0 / l_r[pl.ds(half * 128, 128), :]
            ctx_v[pl.ds(i * RB // 2 + half * 64, 64), cols] = _pk(acc * inv)

    NS, NP = 3, 3
    sbuf, pbuf, lbuf = (s0, s1, s2), (p0, p1, p2), (l0, l1, l2)
    bufa, bufb = (qa, ka, va), (qb, kb, vb)
    wa, wb = (wqa, wka, wva), (wqb, wkb, wvb)

    def projector(w, buf):
        return lambda i: proj(i, w, buf)

    def head_pair(head, fill, unpack_a, unpack_b):
        tasks = [(bufa, head, i) for i in range(NB)] + [(bufb, head + 1, i) for i in reversed(range(NB))]
        n = len(tasks)
        for t in range(max([n + 1] + list(fill)) + 1):
            for f in fill.get(t, ()):
                f()
            if t == 1 and unpack_a is not None:
                unpack_a()
            if t == NB + 1 and unpack_b is not None:
                unpack_b()
            if t < n:
                (q_r, k_r, _), _, i = tasks[t]
                stage_a(i, q_r, k_r, sbuf[t % NS])
            if 1 <= t <= n:
                stage_b(tasks[t - 1][2], sbuf[(t - 1) % NS], pbuf[(t - 1) % NP], lbuf[(t - 1) % NP])
            if 2 <= t < n + 2:
                (_, _, v_r), hd, i = tasks[t - 2]
                stage_c(i, v_r, pbuf[(t - 2) % NP], lbuf[(t - 2) % NP], hd)

    def fills(first, second):
        fill = {0: [functools.partial(first, 0), functools.partial(first, 1)]}
        for i in range(2, NB):
            fill[i - 1] = [functools.partial(first, i)]
        if second is not None:
            for i in range(NB):
                fill[NB + 2 + i] = [functools.partial(second, i)]
        return fill

    c_x.wait()
    for i in range(NB):
        xn_v[pl.ds(i * RB // 2, RB // 2), :] = _pk(_layernorm(x_v[pl.ds(i * RB, RB), :].astype(F32)))
    c_wq[0].wait()
    unpack(wq32, wqa, 0, False, M)
    unpack(wq32, wqb, 0, True, M)
    for i in range(NB):
        rows = pl.ds(i * RB // 2, RB // 2)
        qa[rows, :] = _pk(_nn(_up(xn_v[rows, :]), _up(wqa[...])) * QSCALE)
    c_ckv.wait()
    for i in range(NB):
        ckp_v[pl.ds(i * RB // 2, RB // 2), :] = _pk(ckv_v[pl.ds(i * RB, RB), :])
    c_wuk[0].wait()
    unpack(wuk32, wka, 0, False, DC)
    unpack(wuk32, wkb, 0, True, DC)
    for i in range(NB):
        rows = pl.ds(i * RB // 2, RB // 2)
        ka[rows, :] = _pk(_nn(_up(ckp_v[rows, :]), _up(wka[...])))
    c_wuv[0].wait()
    unpack(wuv32, wva, 0, False, DC)
    unpack(wuv32, wvb, 0, True, DC)
    for i in range(NB):
        rows = pl.ds(i * RB // 2, RB // 2)
        va[rows, :] = _pk(_nn(_up(ckp_v[rows, :]), _up(wva[...])))

    def pair_body(j, carry):
        @pl.when(j == H // 4 - 1)
        def _():
            for c in second:
                c.wait()

        head_pair(2 * j, fills(projector(wb, bufb), projector(wa, bufa)),
                  lambda: unpack_head(j + 1, False, *wa), lambda: unpack_head(j + 1, True, *wb))
        return carry

    lax.fori_loop(0, H // 2 - 1, pair_body, 0)
    for c in late:
        c.wait()
    wr = wr_v[...].astype(F32).reshape(1, M)
    best = {}

    def out_block(i):
        OM = 128
        for r0 in range(i * RB, (i + 1) * RB, OM):
            rows, rows2 = pl.ds(r0, OM), pl.ds(r0 // 2, OM // 2)
            attn = _r16(_nn(_up(ctx_v[rows2, :]), _up(wop_v[...])))
            h = _r16(x_v[rows, :].astype(F32) + attn)
            hn = _r16(_layernorm(h))
            x_v[rows, :] = h.astype(BF16)
            xn_v[rows2, :] = _pk(hn)
            out_v[rows, :] = (h + hn).astype(BF16)
            best[r0] = _r16(jnp.sum(hn * wr, axis=-1, keepdims=True))
        rows = pl.ds(i * RB, RB)
        pltpu.make_async_copy(out_v.at[rows, :], out_h.at[rows, :], sems.at[i]).start()

    def pack_wo():
        for c in range(H * D // 256):
            wop_v[pl.ds(c * 128, 128), :] = _pk(wo_v[pl.ds(c * 256, 256), :])

    fill = fills(projector(wb, bufb), None)
    for u in range(NB):
        fill[NB + 3 + u] = [functools.partial(out_block, NB - 1 - u)]
    head_pair(H - 2, fill, pack_wo, None)
    best = [best[k] for k in sorted(best)]
    r = jnp.concatenate(best, axis=0)
    ridx = lax.broadcasted_iota(jnp.int32, (S, 1), 0)
    r1 = jnp.max(r, axis=0, keepdims=True)
    i1 = jnp.min(jnp.where(r == r1, ridx, S), axis=0, keepdims=True)
    rr = jnp.where(ridx == i1, -jnp.inf, r)
    r2 = jnp.max(rr, axis=0, keepdims=True)
    i2 = jnp.min(jnp.where(rr == r2, ridx, S), axis=0, keepdims=True)
    idx1, idx2 = i1[0, 0], i2[0, 0]

    row16 = lax.broadcasted_iota(jnp.int32, (16, M), 0)
    g1 = pl.multiple_of((idx1 // 16) * 16, 16)
    g2 = pl.multiple_of((idx2 // 16) * 16, 16)
    hn1 = _up(xn_v[pl.ds(pl.multiple_of(g1 // 2, 8), 8), :]).astype(F32)
    hn2 = _up(xn_v[pl.ds(pl.multiple_of(g2 // 2, 8), 8), :]).astype(F32)
    m1, m2 = row16 == idx1 - g1, row16 == idx2 - g2
    x1 = jnp.sum(jnp.where(m1, hn1, 0.0), axis=0, keepdims=True)
    x2 = jnp.sum(jnp.where(m2, hn2, 0.0), axis=0, keepdims=True)
    xs = jnp.where(row16 == 0, x1, jnp.where(row16 == 1, x2, 0.0)).astype(BF16)

    gate = _r16(_nn(xs, wg_v[...]))
    up = _r16(_nn(xs, wu_v[...]))
    act = _r16(_r16(gate * _r16(jax.nn.sigmoid(gate))) * up).astype(BF16)
    y = _r16(_nn(act, wd_v[...]))
    y1 = _r16(y[0:1] * _r16(jax.nn.sigmoid(r1)))
    y2 = _r16(y[1:2] * _r16(jax.nn.sigmoid(r2)))

    for i in range(NB):
        rows = pl.ds(i * RB, RB)
        pltpu.make_async_copy(out_v.at[rows, :], out_h.at[rows, :], sems.at[i]).wait()

    def fix(g, mask, hn, yrow):
        h = x_v[pl.ds(g, 16), :].astype(F32)
        old = out_v[pl.ds(g, 16), :]
        new = (h + _r16(hn + yrow)).astype(BF16)
        out_v[pl.ds(g, 16), :] = jnp.where(mask, new, old)

    fix(g1, m1, hn1, y1)
    fix(g2, m2, hn2, y2)
    c1 = pltpu.make_async_copy(out_v.at[pl.ds(g1, 16), :], out_h.at[pl.ds(g1, 16), :], osem.at[0])
    c1.start()

    @pl.when(g1 != g2)
    def _():
        c2 = pltpu.make_async_copy(out_v.at[pl.ds(g2, 16), :], out_h.at[pl.ds(g2, 16), :], osem.at[1])
        c2.start()
        c2.wait()

    c1.wait()


@jax.jit
def pallas_sequential_preLN__compressed_kv_cla__moe_arch_mod__prompt_kernel(
    A_x: jax.Array,
    A_c_kv: jax.Array,
    A_w_q: jax.Array,
    A_w_uk: jax.Array,
    A_w_uv: jax.Array,
    A_w_o: jax.Array,
    B_x: jax.Array,
    B_w_r: jax.Array,
    B_w_gate: jax.Array,
    B_w_up: jax.Array,
    B_w_down: jax.Array,
):
    del B_x
    hbm = pl.BlockSpec(memory_space=pl.ANY)
    vm = pltpu.VMEM
    u32 = jnp.uint32
    scratch = [
        vm((S, M), BF16), vm((S // 2, M), u32), vm((S, DC), BF16), vm((S // 2, DC), u32),
        vm((2, M, 8, D), u32), vm((2, DC, 8, D), u32), vm((2, DC, 8, D), u32),
        vm((H * D, M), BF16), vm((H * D // 2, M), u32), vm((M,), BF16), vm((M, F), BF16), vm((M, F), BF16), vm((F, M), BF16),
        vm((S // 2, H * D), u32), vm((S, M), BF16),
        vm((M // 2, D), u32), vm((DC // 2, D), u32), vm((DC // 2, D), u32),
        vm((M // 2, D), u32), vm((DC // 2, D), u32), vm((DC // 2, D), u32),
        vm((S // 2, D), u32), vm((S // 2, D), u32), vm((S // 2, D), u32),
        vm((S // 2, D), u32), vm((S // 2, D), u32), vm((S // 2, D), u32),
        vm((RB, S), F32), vm((RB, S), F32), vm((RB, S), F32),
        vm((RB // 2, S), u32), vm((RB // 2, S), u32), vm((RB // 2, S), u32),
        vm((RB, 128), F32), vm((RB, 128), F32), vm((RB, 128), F32),
        pltpu.SMEM((1,), jnp.int32),
        pltpu.SemaphoreType.DMA((13,)), pltpu.SemaphoreType.DMA((2,)),
    ]
    out = pl.pallas_call(
        _kernel,
        out_shape=jax.ShapeDtypeStruct((S, M), BF16),
        in_specs=[hbm] * 10,
        out_specs=hbm,
        scratch_shapes=scratch,
        compiler_params=pltpu.CompilerParams(vmem_limit_bytes=126 * 1024 * 1024),
    )(
        A_x.reshape(S, M), A_c_kv.reshape(S, DC),
        A_w_q.reshape(M, 2, H // 2, D), A_w_uk.reshape(DC, 2, H // 2, D), A_w_uv.reshape(DC, 2, H // 2, D),
        A_w_o.reshape(H * D, M), B_w_r, B_w_gate, B_w_up, B_w_down,
    )
    return out.reshape(1, S, M)
```
